```python
import os as _os
_os.environ.setdefault("JAX_PLATFORMS", "cpu")
import jax
import jax.numpy as jnp

def _softmax(x, axis=-1):
    return jax.nn.softmax(x, axis=axis)
def _gelu(x):
    return jax.nn.gelu(x, approximate=True)
def _silu(x):
    return jax.nn.silu(x)
def _sigmoid(x):
    return jax.nn.sigmoid(x)
def _layernorm(x, axis=-1, eps=1e-5):
    m = jnp.mean(x, axis=axis, keepdims=True)
    v = jnp.var(x, axis=axis, keepdims=True)
    return (x - m) / jnp.sqrt(v + eps)
def _scatter_add(tgt, idx, src, axis=0):
    return tgt.at[idx].add(src)
def _segment_sum(src, seg, n):
    return jax.ops.segment_sum(src, seg, n)
class _Rng:
    def __init__(self, key):
        self._k = key
    def _next(self):
        self._k, sub = jax.random.split(self._k)
        return sub
    def normal(self, shape):
        return jax.random.normal(self._next(), shape, dtype=jnp.bfloat16)
    def randint(self, lo, hi, shape):
        return jax.random.randint(self._next(), shape, lo, hi, dtype=jnp.int32)
    def uniform(self, shape, lo=0.0, hi=1.0):
        return jax.random.uniform(self._next(), shape, jnp.bfloat16, lo, hi)
    def permutation(self, n):
        return jax.random.permutation(self._next(), n)


kernel_name = 'sequential_preLN__linear_kernel_hedgehog__dense_activation_squared_relu__prompt'

def setup_inputs():
    _rng = _Rng(jax.random.key(int.from_bytes(__import__("os").urandom(4), "little")))
    _w = (lambda a: (lambda t: t.astype(jnp.bfloat16) if jnp.issubdtype(t.dtype, jnp.floating) else t)(jnp.asarray(a)))
    def _A_setup():
        B, S, D, H = 1, 2048, 512, 32
        Dh = D // H
        return {
            "x": _w((lambda *s: _rng.normal(s) * 0.05)(B, S, D)),
            "wqkv": _w((lambda *s: _rng.normal(s) * 0.2)(D, 3 * D)),
            "w_phi": _w((lambda *s: _rng.normal(s) * 0.2)(H, Dh, Dh) * (Dh ** -0.5)),
            "wo": _w((lambda *s: _rng.normal(s) * 0.05)(D, D)),
        }
    _A_in = _A_setup()

    def _B_setup():
        B, S, D, F = 1, 2048, 512, 1792
        return {
            "x": _w((lambda *s: _rng.normal(s) * 0.05)(B, S, D)),
            "w1": _w((lambda *s: _rng.normal(s) * 0.05)(D, F)),
            "b1": _w((lambda *s: _rng.normal(s) * 0.05)(F)),
            "w2": _w((lambda *s: _rng.normal(s) * 0.05)(F, D)),
            "b2": _w((lambda *s: _rng.normal(s) * 0.05)(D)),
        }
    _B_in = _B_setup()

    return {
        "A_x": _A_in["x"],
        "A_wqkv": _A_in["wqkv"],
        "A_w_phi": _A_in["w_phi"],
        "A_wo": _A_in["wo"],
        "B_x": _B_in["x"],
        "B_w1": _B_in["w1"],
        "B_b1": _B_in["b1"],
        "B_w2": _B_in["w2"],
        "B_b2": _B_in["b2"],
    }

def reference(A_x, A_wqkv, A_w_phi, A_wo, B_x, B_w1, B_b1, B_w2, B_b2):
    def _A_ref(x, wqkv, w_phi, wo):
        B, S, D = x.shape
        H = 32; Dh = D // H
        qkv = (lambda x, *d: x.transpose(*d))((x @ wqkv).reshape(B, S, 3, H, Dh), 2, 0, 3, 1, 4)
        q, k, v = qkv[0], qkv[1], qkv[2]
        pq = jnp.einsum("bhsd,hdf->bhsf", q, w_phi)
        pk = jnp.einsum("bhsd,hdf->bhsf", k, w_phi)
        phi_q = jnp.concatenate([_softmax(pq, axis=-1), _softmax(-pq, axis=-1)], axis=-1)
        phi_k = jnp.concatenate([_softmax(pk, axis=-1), _softmax(-pk, axis=-1)], axis=-1)
        kv = jnp.einsum("bhsf,bhsd->bhfd", phi_k, v)
        z  = jnp.einsum("bhsf->bhf", phi_k)
        num = jnp.einsum("bhqf,bhfd->bhqd", phi_q, kv)
        den = jnp.einsum("bhqf,bhf->bhq", phi_q, z)[..., None] + 1e-6
        o = num / den
        return (lambda x, *d: x.transpose(*d))(o, 0, 2, 1, 3).reshape(B, S, D) @ wo

    def _B_ref(x, w1, b1, w2, b2):
        h = jnp.einsum("bsd,df->bsf", x, w1) + b1
        zero = jnp.zeros_like(h)
        r = jnp.where(h > zero, h, zero)
        h = r * r
        out = jnp.einsum("bsf,fd->bsd", h, w2) + b2
        return out

    x = A_x
    h = x + _A_ref(_layernorm(x, axis=-1), A_wqkv, A_w_phi, A_wo)
    h2 = h + _B_ref(_layernorm(h, axis=-1), B_w1, B_b1, B_w2, B_b2)
    return h2
```

```python
import jax
import jax.numpy as jnp
from jax import lax
import jax.experimental.pallas as pl
import jax.experimental.pallas.tpu as pltpu

S, D, H, DH, F = 2048, 512, 32, 16, 1792
G8 = 8
EPS = 1e-5

_NT = (((1,), (1,)), ((), ()))


def _layernorm(x):
    m = jnp.mean(x, axis=-1, keepdims=True)
    xc = x - m
    v = jnp.mean(xc * xc, axis=-1, keepdims=True)
    return xc * lax.rsqrt(v + EPS)


def make_kernel(T=512, FC=256, C=256, CA=512, skew=1, TL=128, KS=2, ln2b=0):
    nT = S // T
    nFC = F // FC
    nC = T // C
    X0 = 256

    def kernel(x_hbm, wqkv_hbm, wphi_hbm, wo_hbm, w1_hbm, b1_hbm, w2_hbm, b2_hbm,
               out_hbm,
               x_v, xn_v, wqkv_v, wphi_v, wo_v, w1_v, b1_v, w2_v, b2_v,
               wkt_v, wvt_v, wqt_v, kvt_acc, z_acc, kvt_v, zb_v, h_v, hn_v, out_v,
               sem_x, sem_w, sem_k, sem_o):
        def x_cp(r0, n, k):
            return pltpu.make_async_copy(x_hbm.at[0, pl.ds(r0, n), :],
                                         x_v.at[pl.ds(r0, n), :], sem_x.at[k])
        x0a = x_cp(0, X0, 0)
        x0b = x_cp(X0, T - X0, 1)
        x1 = x_cp(T, T, 2)
        x23 = x_cp(2 * T, S - 2 * T, 3)

        def wcol_cp(c0, n, sem):
            return pltpu.make_async_copy(wqkv_hbm.at[:, pl.ds(c0, n)],
                                         wqkv_v.at[:, pl.ds(c0, n)], sem)
        KW = D // KS
        wk_cp = [wcol_cp(D + u * KW, KW, sem_k.at[u]) for u in range(KS)]
        wq_cp = wcol_cp(0, D, sem_w.at[0])
        wv_cp = wcol_cp(2 * D, D, sem_w.at[2])
        wphi_cp = pltpu.make_async_copy(wphi_hbm, wphi_v, sem_w.at[3])
        wo_cp = pltpu.make_async_copy(wo_hbm, wo_v, sem_w.at[4])
        w1_cp = pltpu.make_async_copy(w1_hbm, w1_v, sem_w.at[5])
        w2_cp = pltpu.make_async_copy(w2_hbm, w2_v, sem_w.at[6])
        b1_cp = pltpu.make_async_copy(b1_hbm, b1_v, sem_w.at[7])
        b2_cp = pltpu.make_async_copy(b2_hbm, b2_v, sem_w.at[8])

        def out_cp(row, n, k):
            return pltpu.make_async_copy(out_v.at[pl.ds(row, n), :],
                                         out_hbm.at[0, pl.ds(row, n), :], sem_o.at[k])

        def rowof(i):
            return i * T if isinstance(i, int) else pl.multiple_of(i * T, T)

        for cp in [wphi_cp, x0a] + wk_cp:
            cp.start()

        def halves(a, op):
            return op(a, pltpu.roll(a, 4, axis=1))

        def feat(pT):
            W = pT.shape[-1]
            p4 = pT.reshape(G8, 8, 8, W)
            mx = halves(jnp.max(p4, axis=1), jnp.maximum)[:, None]
            mn = halves(jnp.min(p4, axis=1), jnp.minimum)[:, None]
            ep = jnp.exp(p4 - mx)
            en = jnp.exp(mn - p4)
            sp = halves(jnp.sum(ep, axis=1), jnp.add)[:, None]
            sn = halves(jnp.sum(en, axis=1), jnp.add)[:, None]
            return ep, en, sp, sn

        def ln1(m):
            r0 = m * C
            xn = _layernorm(x_v[r0:r0 + C, :].astype(jnp.float32)).astype(jnp.bfloat16)
            xn_v[r0:r0 + C, :] = xn
            return xn

        def p1_k(xn):
            pkT = lax.dot_general(wkt_v[...], xn, _NT, preferred_element_type=jnp.float32)
            ep, en, sp, sn = feat(pkT)
            php = (ep * (1.0 / sp)).reshape(G8, 64, C)
            phn = (en * (1.0 / sn)).reshape(G8, 64, C)
            ph = jnp.concatenate([php, phn], axis=1)
            zs = ph[:, :, 0:128]
            for cidx in range(1, C // 128):
                zs = zs + ph[:, :, cidx * 128:(cidx + 1) * 128]
            z_acc[...] += zs
            return ph.astype(jnp.bfloat16)

        def p1_v(xn):
            return lax.dot_general(wvt_v[...], xn, _NT,
                                   preferred_element_type=jnp.float32).astype(jnp.bfloat16)

        def p1_kv(vT, phb):
            for g in range(G8):
                kvt_acc[g] += lax.dot_general(vT[g * 64:(g + 1) * 64, :], phb[g], _NT,
                                              preferred_element_type=jnp.float32)

        if True:
            r = lax.broadcasted_iota(jnp.int32, (H, H * DH), 0)
            c = lax.broadcasted_iota(jnp.int32, (H, H * DH), 1)
            eh = (r == c // DH).astype(jnp.bfloat16)
            r = lax.broadcasted_iota(jnp.int32, (DH * DH, H * DH), 0)
            c = lax.broadcasted_iota(jnp.int32, (DH * DH, H * DH), 1)
            m1 = r // DH == c % DH
            r = lax.broadcasted_iota(jnp.int32, (128, DH * DH), 0)
            c = lax.broadcasted_iota(jnp.int32, (128, DH * DH), 1)
            pm = ((r % 64) // 4 == c % DH).astype(jnp.bfloat16)
            rr = lax.broadcasted_iota(jnp.int32, (128, H * DH), 0)
            cc = lax.broadcasted_iota(jnp.int32, (128, H * DH), 1)
            m2 = (rr // 64) * 4 + rr % 4 == (cc // DH) % 8
            r = lax.broadcasted_iota(jnp.int32, (128, 128), 0)
            c = lax.broadcasted_iota(jnp.int32, (128, 128), 1)
            eye = (r == c).astype(jnp.bfloat16)
            kvt_acc[...] = jnp.zeros_like(kvt_acc)
            z_acc[...] = jnp.zeros_like(z_acc)

            wphi_cp.wait()
            wv_cp.start()
            x0b.start()
            wt2 = wphi_v[...].reshape(DH * DH, H)
            xr = jnp.dot(wt2, eh, preferred_element_type=jnp.float32)
            xm = jnp.where(m1, xr, 0.0).astype(jnp.bfloat16)
            rep = jnp.dot(pm, xm, preferred_element_type=jnp.float32)
            bdt = jnp.where(m2, rep, 0.0).astype(jnp.bfloat16)
            n0 = X0 // C

            def fold(j, dst, gs=range(4)):
                for g in gs:
                    w = wqkv_v[:, j * D + g * 128: j * D + (g + 1) * 128]
                    lhs = eye if j == 2 else bdt[:, g * 128:(g + 1) * 128]
                    dst[g * 128:(g + 1) * 128, :] = lax.dot_general(
                        lhs, w, _NT, preferred_element_type=jnp.float32).astype(jnp.bfloat16)

            gper = 4 // KS
            for u in range(KS):
                wk_cp[u].wait()
                if u == 0:
                    x1.start()
                if u == KS - 1:
                    x0a.wait()
                    wq_cp.start()
                    wo_cp.start()
                fold(1, wkt_v, range(u * gper, (u + 1) * gper))
            xns = [ln1(m) for m in range(n0)]
            phs = [p1_k(xn) for xn in xns]
            wv_cp.wait()
            x0b.wait()
            x23.start()
            fold(2, wvt_v)

        if True:
            pend = [(p1_v(xn), ph) for xn, ph in zip(xns, phs)]
            for m in range(n0, S // C):
                if m == nC or m == 2 * nC:
                    if m == nC:
                        x1.wait()
                        wq_cp.wait()
                        wo_cp.wait()
                        for cp in (w1_cp, w2_cp, b1_cp, b2_cp):
                            cp.start()
                    else:
                        x23.wait()
                    while pend:
                        p1_kv(*pend.pop(0))
                while len(pend) > skew:
                    p1_kv(*pend.pop(0))
                xn = ln1(m)
                ph = p1_k(xn)
                pend.append((p1_v(xn), ph))
                if m == nC:
                    fold(0, wqt_v)
            while pend:
                p1_kv(*pend.pop(0))

        def a_stages(row, W, slot, off):
            st = {}

            def a1():
                xn = xn_v[pl.ds(row, W), :]
                st['pqT'] = lax.dot_general(wqt_v[...], xn, _NT, preferred_element_type=jnp.float32)

            def a2():
                ep, en, sp, sn = feat(st['pqT'])
                zb = zb_v[...]
                zbt = jnp.concatenate([zb] * (W // 128), axis=-1) if W > 128 else zb
                zp = zbt[:, 0:64, :].reshape(G8, 8, 8, W)
                zn = zbt[:, 64:128, :].reshape(G8, 8, 8, W)
                ap = halves(jnp.sum(ep * zp, axis=1), jnp.add)[:, None]
                an = halves(jnp.sum(en * zn, axis=1), jnp.add)[:, None]
                rp = 1.0 / sp
                rn = 1.0 / sn
                den = ap * rp + an * rn + 1e-6
                rd = 1.0 / den
                php = (ep * (rp * rd)).reshape(G8, 64, W)
                phn = (en * (rn * rd)).reshape(G8, 64, W)
                st['ph'] = jnp.concatenate([php, phn], axis=1).astype(jnp.bfloat16)

            def a3():
                ph = st['ph']
                oT = jnp.concatenate(
                    [jnp.dot(kvt_v[g], ph[g], preferred_element_type=jnp.float32) for g in range(G8)],
                    axis=0)
                st['o'] = oT.T.astype(jnp.bfloat16)

            def a4():
                attn = jnp.dot(st['o'], wo_v[...], preferred_element_type=jnp.float32)
                st['h'] = x_v[pl.ds(row, W), :].astype(jnp.float32) + attn

            def a5():
                h = st['h']
                h_v[slot, off:off + W, :] = h
                if not ln2b:
                    hn_v[slot, off:off + W, :] = _layernorm(h).astype(jnp.bfloat16)

            return [a1, a2, a3, a4, a5]

        def b_stages(row, slot, off, W):
            st = {}

            def b0():
                h = h_v[slot, off:off + W, :]
                if ln2b:
                    st['hn'] = _layernorm(h).astype(jnp.bfloat16)
                st['acc'] = h + b2_v[...].astype(jnp.float32).reshape(1, D)
                st['b1'] = b1_v[...].astype(jnp.float32).reshape(1, F)

            def bc(c):
                def f():
                    hn = st['hn'] if ln2b else hn_v[slot, off:off + W, :]
                    h1 = jnp.dot(hn, w1_v[:, c * FC:(c + 1) * FC], preferred_element_type=jnp.float32)
                    h1 = jnp.maximum(h1 + st['b1'][:, c * FC:(c + 1) * FC], 0.0)
                    h2 = (h1 * h1).astype(jnp.bfloat16)
                    st['acc'] = st['acc'] + jnp.dot(h2, w2_v[c * FC:(c + 1) * FC, :],
                                                    preferred_element_type=jnp.float32)
                return f

            def bstore():
                out_v[pl.ds(row, W), :] = st['acc'].astype(jnp.bfloat16)

            return [b0] + [bc(c) for c in range(nFC)], bstore

        if True:
            nCA = T // CA
            As = [a_stages(m * CA, CA, 0, m * CA) for m in range(nCA)]
            As[0][0]()
            kr = lax.broadcasted_iota(jnp.int32, (G8, 64, 128), 1)
            kc = lax.broadcasted_iota(jnp.int32, (G8, 64, 128), 2)
            kvt_v[...] = jnp.where(kr // DH == kc % 4, kvt_acc[...], 0.0).astype(jnp.bfloat16)
            zsum = jnp.sum(z_acc[...], axis=-1, keepdims=True)
            zb_v[...] = jnp.broadcast_to(zsum, (G8, 128, 128))
            nst = 5
            for w in range(nst + nCA - 1):
                for m in range(nCA):
                    k = w - m
                    if 0 <= k < nst and not (m == 0 and k == 0):
                        As[m][k]()
            w1_cp.wait()
            w2_cp.wait()
            b1_cp.wait()
            b2_cp.wait()

            def body(i, carry):
                slot = lax.rem(i, 2)
                A = a_stages(rowof(i + 1), T, 1 - slot, 0)
                B, bstore = b_stages(rowof(i), slot, 0, T)
                if ln2b:
                    seq = [A[0], B[0]]
                    k = 1
                else:
                    seq = [B[0]]
                    k = 0
                for f in B[1:]:
                    seq.append(f)
                    if k < len(A):
                        seq.append(A[k]); k += 1
                seq += A[k:]
                for f in seq:
                    f()
                bstore()
                out_cp(rowof(i), T, i).start()
                return carry

            lax.fori_loop(0, nT - 1, body, 0)
            i = nT - 1
            slot = i % 2
            parts = [(0, T - TL), (T - TL, TL)] if TL else [(0, T)]
            for k, (off, W) in enumerate(parts):
                B, bstore = b_stages(rowof(i) + off, slot, off, W)
                for f in B:
                    f()
                bstore()
                out_cp(rowof(i) + off, W, i + k).start()
        if True:
            for j in range(nT - 1):
                out_cp(rowof(j), T, j).wait()
            for k, (off, W) in enumerate(parts):
                out_cp(rowof(i) + off, W, i + k).wait()

    def fn(A_x, A_wqkv, A_w_phi, A_wo, B_x, B_w1, B_b1, B_w2, B_b2):
        bf = jnp.bfloat16
        any_spec = pl.BlockSpec(memory_space=pl.ANY)
        wphi_t = jnp.transpose(A_w_phi, (1, 2, 0))
        return pl.pallas_call(
            kernel,
            out_shape=jax.ShapeDtypeStruct((1, S, D), bf),
            in_specs=[any_spec] * 8,
            out_specs=any_spec,
            scratch_shapes=[
                pltpu.VMEM((S, D), bf),
                pltpu.VMEM((S, D), bf),
                pltpu.VMEM((D, 3 * D), bf),
                pltpu.VMEM((DH, DH, H), bf),
                pltpu.VMEM((D, D), bf),
                pltpu.VMEM((D, F), bf),
                pltpu.VMEM((F,), bf),
                pltpu.VMEM((F, D), bf),
                pltpu.VMEM((D,), bf),
                pltpu.VMEM((D, D), bf),
                pltpu.VMEM((D, D), bf),
                pltpu.VMEM((D, D), bf),
                pltpu.VMEM((G8, 64, 128), jnp.float32),
                pltpu.VMEM((G8, 128, 128), jnp.float32),
                pltpu.VMEM((G8, 64, 128), bf),
                pltpu.VMEM((G8, 128, 128), jnp.float32),
                pltpu.VMEM((2, T, D), jnp.float32),
                pltpu.VMEM((2, T, D), bf),
                pltpu.VMEM((S, D), bf),
                pltpu.SemaphoreType.DMA((4,)),
                pltpu.SemaphoreType.DMA((9,)),
                pltpu.SemaphoreType.DMA((4,)),
                pltpu.SemaphoreType.DMA((nT + 1,)),
            ],
            compiler_params=pltpu.CompilerParams(vmem_limit_bytes=100 * 1024 * 1024),
        )(A_x, A_wqkv, wphi_t, A_wo, B_w1, B_b1, B_w2, B_b2)

    return fn


pallas_sequential_preLN__linear_kernel_hedgehog__dense_activation_squared_relu__prompt_kernel = jax.jit(make_kernel())
```

```python
import jax
import jax.numpy as jnp
from jax import lax
import jax.experimental.pallas as pl
import jax.experimental.pallas.tpu as pltpu

S, D, H, DH, F = 2048, 512, 32, 16, 1792
G8 = 8
EPS = 1e-5
LOG2E = 1.4426950408889634

T = 512
FC = 256
C = 256
SKEW = 1
TL = 128
X0 = 256
X1 = 512
KW = D // 2
NT_ = S // T
NFC = F // FC

_NT = (((1,), (1,)), ((), ()))


def _layernorm(x):
    m = jnp.mean(x, axis=-1, keepdims=True)
    xc = x - m
    v = jnp.mean(xc * xc, axis=-1, keepdims=True)
    return xc * lax.rsqrt(v + EPS)


def _halves(a, op):
    return op(a, pltpu.roll(a, 4, axis=1))


def _feat(pT):
    W = pT.shape[-1]
    p4 = pT.reshape(G8, 8, 8, W)
    mx = _halves(jnp.max(p4, axis=1), jnp.maximum)[:, None]
    mn = _halves(jnp.min(p4, axis=1), jnp.minimum)[:, None]
    ep = jnp.exp2(p4 - mx)
    en = jnp.exp2(mn - p4)
    sp = _halves(jnp.sum(ep, axis=1), jnp.add)[:, None]
    sn = _halves(jnp.sum(en, axis=1), jnp.add)[:, None]
    return ep, en, sp, sn


def _kernel(x_hbm, wqkv_hbm, wphi_hbm, wo_hbm, w1_hbm, b1_hbm, w2_hbm, b2_hbm,
            out_hbm,
            x_v, xn_v, wq_v, wk0_v, wk1_v, wv_v, wphi_v, wo_v, w1_v, b1_v, w2_v, b2_v,
            wkt_v, wvt_v, wqt_v, kvt_acc, z_acc, kvt_v, zb_v, h_v, hn_v, out_v,
            sem_x, sem_w, sem_o):
    f32, bf16 = jnp.float32, jnp.bfloat16

    def x_cp(r0, n, k):
        return pltpu.make_async_copy(x_hbm.at[0, pl.ds(r0, n), :],
                                     x_v.at[pl.ds(r0, n), :], sem_x.at[k])
    x0a = x_cp(0, X0, 0)
    x0b = x_cp(X0, X1, 1)
    xr = x_cp(X0 + X1, S - X0 - X1, 2)

    def wcol_cp(c0, n, dst, k):
        return pltpu.make_async_copy(wqkv_hbm.at[:, pl.ds(c0, n)], dst, sem_w.at[k])
    wq_cp = wcol_cp(0, D, wq_v, 0)
    wk0_cp = wcol_cp(D, KW, wk0_v, 1)
    wk1_cp = wcol_cp(D + KW, KW, wk1_v, 9)
    wv_cp = wcol_cp(2 * D, D, wv_v, 2)
    wphi_cp = pltpu.make_async_copy(wphi_hbm, wphi_v, sem_w.at[3])
    wo_cp = pltpu.make_async_copy(wo_hbm, wo_v, sem_w.at[4])
    w1_cp = pltpu.make_async_copy(w1_hbm, w1_v, sem_w.at[5])
    w2_cp = pltpu.make_async_copy(w2_hbm, w2_v, sem_w.at[6])
    b1_cp = pltpu.make_async_copy(b1_hbm, b1_v, sem_w.at[7])
    b2_cp = pltpu.make_async_copy(b2_hbm, b2_v, sem_w.at[8])

    def out_cp(row, n, k):
        return pltpu.make_async_copy(out_v.at[pl.ds(row, n), :],
                                     out_hbm.at[0, pl.ds(row, n), :], sem_o.at[k])

    def rowof(i):
        return i * T if isinstance(i, int) else pl.multiple_of(i * T, T)

    for cp in (wphi_cp, x0a, wk0_cp, wk1_cp):
        cp.start()

    def ln1(m):
        r0 = m * C
        xn = _layernorm(x_v[r0:r0 + C, :].astype(f32)).astype(bf16)
        xn_v[r0:r0 + C, :] = xn
        return xn

    def p1_k(xn):
        pkT = lax.dot_general(wkt_v[...], xn, _NT, preferred_element_type=f32)
        ep, en, sp, sn = _feat(pkT)
        php = (ep * (1.0 / sp)).reshape(G8, 64, C)
        phn = (en * (1.0 / sn)).reshape(G8, 64, C)
        ph = jnp.concatenate([php, phn], axis=1)
        zs = ph[:, :, 0:128]
        for cidx in range(1, C // 128):
            zs = zs + ph[:, :, cidx * 128:(cidx + 1) * 128]
        z_acc[...] += zs
        return ph.astype(bf16)

    def p1_v(xn):
        return lax.dot_general(wvt_v[...], xn, _NT, preferred_element_type=f32).astype(bf16)

    def p1_kv(vT, phb):
        for g in range(G8):
            kvt_acc[g] += lax.dot_general(vT[g * 64:(g + 1) * 64, :], phb[g], _NT,
                                          preferred_element_type=f32)

    def a_stages(row, W, slot):
        st = {}

        def a1():
            xn = xn_v[pl.ds(row, W), :]
            st['pqT'] = lax.dot_general(wqt_v[...], xn, _NT, preferred_element_type=f32)

        def a2():
            ep, en, sp, sn = _feat(st['pqT'])
            zbt = jnp.concatenate([zb_v[...]] * (W // 128), axis=-1)
            zp = zbt[:, 0:64, :].reshape(G8, 8, 8, W)
            zn = zbt[:, 64:128, :].reshape(G8, 8, 8, W)
            ap = _halves(jnp.sum(ep * zp, axis=1), jnp.add)[:, None]
            an = _halves(jnp.sum(en * zn, axis=1), jnp.add)[:, None]
            rp = 1.0 / sp
            rn = 1.0 / sn
            den = ap * rp + an * rn + 1e-6
            rd = 1.0 / den
            php = (ep * (rp * rd)).reshape(G8, 64, W)
            phn = (en * (rn * rd)).reshape(G8, 64, W)
            st['ph'] = jnp.concatenate([php, phn], axis=1).astype(bf16)

        def a3():
            ph = st['ph']
            oT = jnp.concatenate(
                [jnp.dot(kvt_v[g], ph[g], preferred_element_type=f32) for g in range(G8)],
                axis=0)
            st['o'] = oT.T.astype(bf16)

        def a4():
            attn = jnp.dot(st['o'], wo_v[...], preferred_element_type=f32)
            st['h'] = x_v[pl.ds(row, W), :].astype(f32) + attn

        def a5():
            h = st['h']
            h_v[slot] = h
            hn_v[slot] = _layernorm(h).astype(bf16)

        return [a1, a2, a3, a4, a5]

    def b_stages(row, slot, off, W):
        st = {}

        def b0():
            st['acc'] = h_v[slot, off:off + W, :] + b2_v[...].astype(f32).reshape(1, D)
            st['b1'] = b1_v[...].astype(f32).reshape(1, F)

        def bc(c):
            def f():
                hn = hn_v[slot, off:off + W, :]
                h1 = jnp.dot(hn, w1_v[:, c * FC:(c + 1) * FC], preferred_element_type=f32)
                h1 = jnp.maximum(h1 + st['b1'][:, c * FC:(c + 1) * FC], 0.0)
                h2 = (h1 * h1).astype(bf16)
                st['acc'] = st['acc'] + jnp.dot(h2, w2_v[c * FC:(c + 1) * FC, :],
                                                preferred_element_type=f32)
            return f

        def bstore():
            out_v[pl.ds(row, W), :] = st['acc'].astype(bf16)

        return [b0] + [bc(c) for c in range(NFC)], bstore

    r = lax.broadcasted_iota(jnp.int32, (H, H * DH), 0)
    c = lax.broadcasted_iota(jnp.int32, (H, H * DH), 1)
    eh = (r == c // DH).astype(bf16)
    r = lax.broadcasted_iota(jnp.int32, (DH * DH, H * DH), 0)
    c = lax.broadcasted_iota(jnp.int32, (DH * DH, H * DH), 1)
    m1 = r // DH == c % DH
    r = lax.broadcasted_iota(jnp.int32, (128, DH * DH), 0)
    c = lax.broadcasted_iota(jnp.int32, (128, DH * DH), 1)
    pm = ((r % 64) // 4 == c % DH).astype(bf16)
    rr = lax.broadcasted_iota(jnp.int32, (128, H * DH), 0)
    cc = lax.broadcasted_iota(jnp.int32, (128, H * DH), 1)
    m2 = (rr // 64) * 4 + rr % 4 == (cc // DH) % 8
    r = lax.broadcasted_iota(jnp.int32, (128, 128), 0)
    c = lax.broadcasted_iota(jnp.int32, (128, 128), 1)
    eye = (r == c).astype(bf16)
    kvt_acc[...] = jnp.zeros_like(kvt_acc)
    z_acc[...] = jnp.zeros_like(z_acc)

    wphi_cp.wait()
    wv_cp.start()
    x0b.start()
    wt2 = wphi_v[...].reshape(DH * DH, H)
    xrp = jnp.dot(wt2, eh, preferred_element_type=f32)
    xm = jnp.where(m1, xrp, 0.0).astype(bf16)
    rep = jnp.dot(pm, xm, preferred_element_type=f32)
    bdt = jnp.where(m2, rep, 0.0).astype(bf16)

    def fold(src, g0, dst, use_eye=False):
        for gl in range(src.shape[1] // 128):
            g = g0 + gl
            w = src[:, gl * 128:(gl + 1) * 128]
            lhs = eye if use_eye else bdt[:, g * 128:(g + 1) * 128]
            res = lax.dot_general(lhs, w, _NT, preferred_element_type=f32)
            if not use_eye:
                res = res * LOG2E
            dst[g * 128:(g + 1) * 128, :] = res.astype(bf16)

    n0 = X0 // C
    wk0_cp.wait()
    xr.start()
    fold(wk0_v, 0, wkt_v)
    wk1_cp.wait()
    x0a.wait()
    wq_cp.start()
    wo_cp.start()
    fold(wk1_v, 2, wkt_v)
    xns = [ln1(m) for m in range(n0)]
    first = [p1_k(xn) for xn in xns]
    wv_cp.wait()
    x0b.wait()
    fold(wv_v, 0, wvt_v, True)

    A0 = a_stages(0, T, 0)
    mb = (X0 + X1) // C
    pend = [(p1_v(xn), ph) for xn, ph in zip(xns, first)]
    for m in range(n0, S // C):
        if m == mb:
            xr.wait()
            wq_cp.wait()
            wo_cp.wait()
            for cp in (w1_cp, w2_cp, b1_cp, b2_cp):
                cp.start()
            while pend:
                p1_kv(*pend.pop(0))
            fold(wq_v, 0, wqt_v)
        while len(pend) > SKEW:
            p1_kv(*pend.pop(0))
        xn = ln1(m)
        ph = p1_k(xn)
        pend.append((p1_v(xn), ph))
    A0[0]()
    while pend:
        p1_kv(*pend.pop(0))

    kr = lax.broadcasted_iota(jnp.int32, (G8, 64, 128), 1)
    kc = lax.broadcasted_iota(jnp.int32, (G8, 64, 128), 2)
    kvt_v[...] = jnp.where(kr // DH == kc % 4, kvt_acc[...], 0.0).astype(bf16)
    zsum = jnp.sum(z_acc[...], axis=-1, keepdims=True)
    zb_v[...] = jnp.broadcast_to(zsum, (G8, 128, 128))

    for f in A0[1:]:
        f()
    w1_cp.wait()
    w2_cp.wait()
    b1_cp.wait()
    b2_cp.wait()

    def body(i, carry):
        slot = lax.rem(i, 2)
        A = a_stages(rowof(i + 1), T, 1 - slot)
        B, bstore = b_stages(rowof(i), slot, 0, T)
        B[0]()
        for cidx in range(1, NFC + 1):
            B[cidx]()
            if cidx <= len(A):
                A[cidx - 1]()
        bstore()
        out_cp(rowof(i), T, i).start()
        return carry

    lax.fori_loop(0, NT_ - 1, body, 0)

    last = NT_ - 1
    parts = [(0, T - TL), (T - TL, TL)]
    for k, (off, W) in enumerate(parts):
        B, bstore = b_stages(rowof(last) + off, last % 2, off, W)
        for f in B:
            f()
        bstore()
        out_cp(rowof(last) + off, W, last + k).start()

    for j in range(NT_ - 1):
        out_cp(rowof(j), T, j).wait()
    for k, (off, W) in enumerate(parts):
        out_cp(rowof(last) + off, W, last + k).wait()


@jax.jit
def pallas_sequential_preLN__linear_kernel_hedgehog__dense_activation_squared_relu__prompt_kernel(
    A_x: jax.Array,
    A_wqkv: jax.Array,
    A_w_phi: jax.Array,
    A_wo: jax.Array,
    B_x: jax.Array,
    B_w1: jax.Array,
    B_b1: jax.Array,
    B_w2: jax.Array,
    B_b2: jax.Array,
):
    del B_x
    bf = jnp.bfloat16
    f32 = jnp.float32
    any_spec = pl.BlockSpec(memory_space=pl.ANY)
    wphi_t = jnp.transpose(A_w_phi, (1, 2, 0))
    return pl.pallas_call(
        _kernel,
        out_shape=jax.ShapeDtypeStruct((1, S, D), bf),
        in_specs=[any_spec] * 8,
        out_specs=any_spec,
        scratch_shapes=[
            pltpu.VMEM((S, D), bf),
            pltpu.VMEM((S, D), bf),
            pltpu.VMEM((D, D), bf),
            pltpu.VMEM((D, KW), bf),
            pltpu.VMEM((D, KW), bf),
            pltpu.VMEM((D, D), bf),
            pltpu.VMEM((DH, DH, H), bf),
            pltpu.VMEM((D, D), bf),
            pltpu.VMEM((D, F), bf),
            pltpu.VMEM((F,), bf),
            pltpu.VMEM((F, D), bf),
            pltpu.VMEM((D,), bf),
            pltpu.VMEM((D, D), bf),
            pltpu.VMEM((D, D), bf),
            pltpu.VMEM((D, D), bf),
            pltpu.VMEM((G8, 64, 128), f32),
            pltpu.VMEM((G8, 128, 128), f32),
            pltpu.VMEM((G8, 64, 128), bf),
            pltpu.VMEM((G8, 128, 128), f32),
            pltpu.VMEM((2, T, D), f32),
            pltpu.VMEM((2, T, D), bf),
            pltpu.VMEM((S, D), bf),
            pltpu.SemaphoreType.DMA((3,)),
            pltpu.SemaphoreType.DMA((10,)),
            pltpu.SemaphoreType.DMA((NT_ + 1,)),
        ],
        compiler_params=pltpu.CompilerParams(
            vmem_limit_bytes=100 * 1024 * 1024,
            disable_bounds_checks=True,
            disable_semaphore_checks=True,
        ),
    )(A_x, A_wqkv, wphi_t, A_wo, B_w1, B_b1, B_w2, B_b2)
```
